```python
import os as _os
_os.environ.setdefault("JAX_PLATFORMS", "cpu")
import jax
import jax.numpy as jnp

def _softmax(x, axis=-1):
    return jax.nn.softmax(x, axis=axis)
def _gelu(x):
    return jax.nn.gelu(x, approximate=True)
def _silu(x):
    return jax.nn.silu(x)
def _sigmoid(x):
    return jax.nn.sigmoid(x)
def _layernorm(x, axis=-1, eps=1e-5):
    m = jnp.mean(x, axis=axis, keepdims=True)
    v = jnp.var(x, axis=axis, keepdims=True)
    return (x - m) / jnp.sqrt(v + eps)
def _scatter_add(tgt, idx, src, axis=0):
    return tgt.at[idx].add(src)
def _segment_sum(src, seg, n):
    return jax.ops.segment_sum(src, seg, n)
class _Rng:
    def __init__(self, key):
        self._k = key
    def _next(self):
        self._k, sub = jax.random.split(self._k)
        return sub
    def normal(self, shape):
        return jax.random.normal(self._next(), shape, dtype=jnp.bfloat16)
    def randint(self, lo, hi, shape):
        return jax.random.randint(self._next(), shape, lo, hi, dtype=jnp.int32)
    def uniform(self, shape, lo=0.0, hi=1.0):
        return jax.random.uniform(self._next(), shape, jnp.bfloat16, lo, hi)
    def permutation(self, n):
        return jax.random.permutation(self._next(), n)


kernel_name = 'concat_heads__gqa_block_cached__gqa_block_cached__decode'

def setup_inputs():
    _rng = _Rng(jax.random.key(int.from_bytes(__import__("os").urandom(4), "little")))
    _w = (lambda a: (lambda t: t.astype(jnp.bfloat16) if jnp.issubdtype(t.dtype, jnp.floating) else t)(jnp.asarray(a)))
    def _A_setup():
        B, Sq, D = 2, 1, 576
        Hq, Hkv, Sk, Dh = 32, 16, 4096, 128
        assert Hq % Hkv == 0, (Hq, Hkv)
        return {
            "x": _w((lambda *s: _rng.normal(s) * 0.8)(B, Sq, D)),
            "k_cache": _w((lambda *s: _rng.normal(s) * 0.8)(B, Hkv, Sk, Dh)),
            "v_cache": _w((lambda *s: _rng.normal(s) * 0.05)(B, Hkv, Sk, Dh)),
            "wq": _w((lambda *s: _rng.normal(s) * 0.8)(D, Hq * Dh) * (D ** -0.5)),
            "wo": _w((lambda *s: _rng.normal(s) * 0.05)(Hq * Dh, D) * ((Hq * Dh) ** -0.5)),
        }
    _A_in = _A_setup()

    def _B_setup():
        B, Sq, D = 2, 1, 576
        Hq, Hkv, Sk, Dh = 32, 16, 4096, 128
        assert Hq % Hkv == 0, (Hq, Hkv)
        return {
            "x": _w((lambda *s: _rng.normal(s) * 0.8)(B, Sq, D)),
            "k_cache": _w((lambda *s: _rng.normal(s) * 0.8)(B, Hkv, Sk, Dh)),
            "v_cache": _w((lambda *s: _rng.normal(s) * 0.05)(B, Hkv, Sk, Dh)),
            "wq": _w((lambda *s: _rng.normal(s) * 0.8)(D, Hq * Dh) * (D ** -0.5)),
            "wo": _w((lambda *s: _rng.normal(s) * 0.05)(Hq * Dh, D) * ((Hq * Dh) ** -0.5)),
        }
    _B_in = _B_setup()

    return {
        "A_x": _A_in["x"],
        "A_k_cache": _A_in["k_cache"],
        "A_v_cache": _A_in["v_cache"],
        "A_wq": _A_in["wq"],
        "A_wo": _A_in["wo"],
        "B_x": _B_in["x"],
        "B_k_cache": _B_in["k_cache"],
        "B_v_cache": _B_in["v_cache"],
        "B_wq": _B_in["wq"],
        "B_wo": _B_in["wo"],
    }

def reference(A_x, A_k_cache, A_v_cache, A_wq, A_wo, B_x, B_k_cache, B_v_cache, B_wq, B_wo):
    def _A_ref(x, k_cache, v_cache, wq, wo):
        B, Sq, D = x.shape
        Hq, Dh = 32, 128
        Hkv = k_cache.shape[1]
        rep = Hq // Hkv
        q = (lambda x, *d: x.transpose(*d))((x @ wq).reshape(B, Sq, Hq, Dh), 0, 2, 1, 3)
        k = jnp.repeat(k_cache, rep, axis=1)
        v = jnp.repeat(v_cache, rep, axis=1)
        scores = jnp.einsum("bhqd,bhkd->bhqk", q, k) * (Dh ** -0.5)
        p = _softmax(scores, axis=-1)
        o = jnp.einsum("bhqk,bhkd->bhqd", p, v)
        return (lambda x, *d: x.transpose(*d))(o, 0, 2, 1, 3).reshape(B, Sq, Hq * Dh) @ wo

    def _B_ref(x, k_cache, v_cache, wq, wo):
        B, Sq, D = x.shape
        Hq, Dh = 32, 128
        Hkv = k_cache.shape[1]
        rep = Hq // Hkv
        q = (lambda x, *d: x.transpose(*d))((x @ wq).reshape(B, Sq, Hq, Dh), 0, 2, 1, 3)
        k = jnp.repeat(k_cache, rep, axis=1)
        v = jnp.repeat(v_cache, rep, axis=1)
        scores = jnp.einsum("bhqd,bhkd->bhqk", q, k) * (Dh ** -0.5)
        p = _softmax(scores, axis=-1)
        o = jnp.einsum("bhqk,bhkd->bhqd", p, v)
        return (lambda x, *d: x.transpose(*d))(o, 0, 2, 1, 3).reshape(B, Sq, Hq * Dh) @ wo

    a = _A_ref(A_x, A_k_cache, A_v_cache, A_wq, A_wo)
    b = _B_ref(B_x, B_k_cache, B_v_cache, B_wq, B_wo)
    return jnp.concatenate([a, b], axis=-1)
```

```python
import numpy as np
import jax
import jax.numpy as jnp
import jax.experimental.pallas as pl
import jax.experimental.pallas.tpu as pltpu

B, D, HQ, HKV, SK, DH = 2, 576, 32, 16, 4096, 128
NT = (((1,), (1,)), ((), ()))
F32, BF16 = jnp.float32, jnp.bfloat16


class Issuer:
    def __init__(self, starts, points):
        self.starts, self.points, self.k, self.done = starts, points, 0, 0

    def __call__(self):
        self.k += 1
        upto = min(len(self.starts), -(-len(self.starts) * self.k // self.points))
        for s in self.starts[self.done:upto]:
            s()
        self.done = upto


def build(SR=256, rows=32, pre=2, compute=True, inter=True, P=6, npc=2, tail=(256,) * 4,
          extra=1, aord=(0, 1, 2, 3), flags=None, mid=0, tshape=(8, 6)):
    SH = 4
    G = 2 * SH
    GW = G * DH
    ngrp = HKV // SH
    nhg = B * ngrp
    nr = SK // SR
    nst = nhg * nr
    L = pre + ngrp
    win = L + extra
    R = D // P
    scale = DH ** -0.5
    ny = R // 8
    assert L == 6 and sum(tail) == GW
    chunks = [(g * GW, GW) for g in range(ngrp - 1)]
    off = (ngrp - 1) * GW
    for t in tail:
        chunks.append((off, t))
        off += t

    def kernel(ax, ak, av, awq, awo, bx, bk, bv, bwq, bwo, out_ref,
               xbuf, wqbuf, wobuf, kvbuf, q_scr, o_scr, xsem, wqsem, wosem, kvsem):
        kv = (ak, av, bk, bv)

        def kv_starts(j):
            slot = jax.lax.rem(j, win)
            h0 = jax.lax.div(j, nr) * SH
            r0 = pl.multiple_of(jax.lax.rem(j, nr) * SR, SR)
            out = []
            for r in range(SR // rows):
                for a in aord:
                    def go(a=a, r=r, p=len(out) % 2):
                        pltpu.make_async_copy(
                            kv[a].at[pl.ds(h0, SH), pl.ds(r0 + r * rows, rows)],
                            kvbuf.at[slot, a, :, pl.ds(r * rows, rows)],
                            kvsem.at[slot]).start(priority=p)
                    out.append(go)
            return out

        def w_starts(src, dst, sem, blocks, n=npc):
            out = []
            for y, ry, x, cx in blocks:
                for p in range(0, P, n):
                    for br in range(2):
                        def go(y=y, ry=ry, x=x, cx=cx, p=p, br=br):
                            idx = (pl.ds(p, n), pl.ds(y, ry), pl.ds(x, cx))
                            pltpu.make_async_copy(src[br].at[idx], dst.at[br].at[idx], sem).start(priority=br)
                        out.append(go)
            return out

        xc = [pltpu.make_async_copy(x, xbuf.at[i], xsem.at[i]) for i, x in enumerate((ax, bx))]
        for i, c in enumerate(xc):
            c.start(priority=i)

        @pl.loop(0, ny)
        def _(i):
            y = pl.multiple_of(i * 8, 8)
            for s in w_starts((awq, bwq), wqbuf, wqsem.at[0], [(y, 8, x, GW) for x in range(0, HQ * DH, GW)]):
                s()

        @pl.loop(0, pre)
        def _(j):
            for s in kv_starts(j):
                s()

        for c in xc:
            c.wait()
        pltpu.make_async_copy(wqbuf, wqbuf, wqsem.at[0]).wait()

        row = jax.lax.broadcasted_iota(jnp.int32, (B * G, DH), 0)
        rowd = jax.lax.broadcasted_iota(jnp.int32, (B * G, D), 0)
        xr = []
        for br in range(2):
            x = xbuf[br].astype(F32)
            xr.append(jnp.where(rowd < G, x[0:1, :], x[1:2, :]).astype(BF16))

        @pl.loop(0, ngrp)
        def _(g):
            issue = Issuer(kv_starts(pre + g), 2 * G if inter else 1)
            if not inter or not compute:
                for _ in range(issue.points):
                    issue()
            if compute:
                for br in range(2):
                    qg = None
                    for t in range(G):
                        c = pl.multiple_of(g * GW + t * DH, DH)
                        w = wqbuf[br, :, :, pl.ds(c, DH)].reshape(D, DH)
                        r = jnp.dot(xr[br], w, preferred_element_type=F32)
                        qg = r if qg is None else jnp.where(row % G == t, r, qg)
                        if inter:
                            issue()
                    for b in range(B):
                        q_scr[br, b * ngrp + g] = qg[b * G:(b + 1) * G]

        def attend(j, carry, starts):
            slot = jax.lax.rem(j, win)
            hg = jax.lax.div(j, nr)
            first = jax.lax.rem(j, nr) == 0
            issue = Issuer(starts, 4 * SH if inter else 1)
            if not inter or not compute:
                for _ in range(issue.points):
                    issue()
            pltpu.make_async_copy(kvbuf.at[slot], kvbuf.at[slot], kvsem.at[slot]).wait()
            if not compute:
                return carry
            hs = jax.lax.broadcasted_iota(jnp.int32, (G, SR), 0) // 2
            ho = jax.lax.broadcasted_iota(jnp.int32, (G, DH), 0) // 2
            ss = []
            for br in range(2):
                q = q_scr[br, hg].astype(BF16)
                s = None
                for h in range(SH):
                    r = jax.lax.dot_general(q, kvbuf[slot, 2 * br, h], NT, preferred_element_type=F32)
                    s = r if s is None else jnp.where(hs == h, r, s)
                    if inter:
                        issue()
                ss.append(s * scale)
            new = []
            for br in range(2):
                m_old, l_old, a_old = carry[br]
                m_old = jnp.where(first, -jnp.inf, m_old)
                l_old = jnp.where(first, 0.0, l_old)
                a_old = jnp.where(first, 0.0, a_old)
                s = ss[br]
                m_new = jnp.maximum(m_old, jnp.max(s, axis=1, keepdims=True))
                alpha = jnp.exp(m_old - m_new)
                ps = [jnp.exp(s[:, t * DH:(t + 1) * DH] - m_new) for t in range(SR // DH)]
                l_new = alpha * l_old + sum(ps[1:], ps[0])
                pb = jnp.concatenate(ps, axis=1).astype(BF16)
                o = None
                for h in range(SH):
                    r = jnp.dot(pb, kvbuf[slot, 2 * br + 1, h], preferred_element_type=F32)
                    o = r if o is None else jnp.where(ho == h, r, o)
                    if inter:
                        issue()
                a_new = alpha * a_old + o
                o_scr[br, hg] = a_new / jnp.sum(l_new, axis=1, keepdims=True)
                new.append((m_new, l_new, a_new))
            return tuple(new)

        z = jnp.zeros((G, DH), F32)
        carry = jax.lax.fori_loop(0, nst - L, lambda j, c: attend(j, c, kv_starts(j + L)), ((z, z, z),) * 2)

        wo = (awo, bwo)

        def body_b(i, c):
            g = jax.lax.div(i, 3)
            x = pl.multiple_of(g * GW, GW)
            y0 = jax.lax.rem(i, 3) * (R // 3)
            blocks = [(pl.multiple_of(y0 + y, 8), 8, x, GW) for y in range(0, R // 3, 8)]
            return attend(nst - L + i, c, w_starts(wo, wobuf, wosem.at[g], blocks))
        jax.lax.fori_loop(0, L, body_b, carry)

        def chunk_starts(i):
            x, cx = chunks[i]
            if cx == GW:
                return w_starts(wo, wobuf, wosem.at[i], [(y, 8, x, cx) for y in range(0, R, 8)])
            ry, n = tshape
            return w_starts(wo, wobuf, wosem.at[i], [(y, ry, x, cx) for y in range(0, R, ry)], n)

        def project(acc, sem, g, t0, nt, starts):
            x = pl.multiple_of(g * GW + t0 * DH, DH)
            issue = Issuer(starts, 2 * nt if inter else 1)
            if not inter or not compute:
                for _ in range(issue.points):
                    issue()
            blk = wobuf.at[:, :, :, pl.ds(x, nt * DH)]
            pltpu.make_async_copy(blk, blk, sem).wait()
            if not compute:
                return acc
            new = []
            for br in range(2):
                og = jnp.concatenate([o_scr[br, b * ngrp + g] for b in range(B)], axis=0)
                a = acc[br]
                for t in range(nt):
                    lhs = jnp.where(row % G == t0 + t, og, 0.0).astype(BF16)
                    w = wobuf[br, :, :, pl.ds(pl.multiple_of(x + t * DH, DH), DH)].reshape(D, DH)
                    a = a + jax.lax.dot_general(lhs, w, NT, preferred_element_type=F32)
                    if inter:
                        issue()
                new.append(a)
            return tuple(new)

        acc = (jnp.zeros((B * G, D), F32),) * 2
        acc = project(acc, wosem.at[0], 0, 0, G, chunk_starts(2))
        acc = project(acc, wosem.at[1], 1, 0, G, sum((chunk_starts(k) for k in range(3, len(chunks))), []))
        nt = tail[0] // DH
        if mid == 0:
            acc = project(acc, wosem.at[2], 2, 0, G, [])
        else:
            acc = jax.lax.fori_loop(2, 3, lambda i, a: project(a, wosem.at[i], i, 0, G, []), acc)
        acc = jax.lax.fori_loop(0, len(tail), lambda i, a: project(a, wosem.at[3 + i], 3, i * nt, nt, []), acc)
        res = jnp.concatenate(acc, axis=1)
        res = jnp.concatenate([jnp.sum(res[b * G:(b + 1) * G], axis=0, keepdims=True) for b in range(B)], axis=0)
        out_ref[...] = res.astype(out_ref.dtype)

    def f(ax, ak, av, awq, awo, bx, bk, bv, bwq, bwo):
        def r(t):
            return t.reshape(B * HKV, SK, DH)

        def w(t):
            return t.reshape(P, R, HQ * DH)
        hbm = pl.BlockSpec(memory_space=pltpu.HBM)
        out = pl.pallas_call(
            kernel,
            out_shape=jax.ShapeDtypeStruct((B, 2 * D), BF16),
            in_specs=[hbm] * 10,
            scratch_shapes=[
                pltpu.VMEM((2, B, D), BF16),
                pltpu.VMEM((2, P, R, HQ * DH), BF16),
                pltpu.VMEM((2, P, R, HQ * DH), BF16),
                pltpu.VMEM((win, 4, SH, SR, DH), BF16),
                pltpu.VMEM((2, nhg, G, DH), F32),
                pltpu.VMEM((2, nhg, G, DH), F32),
                pltpu.SemaphoreType.DMA((2,)),
                pltpu.SemaphoreType.DMA((1,)),
                pltpu.SemaphoreType.DMA((len(chunks),)),
                pltpu.SemaphoreType.DMA((win,)),
            ],
            compiler_params=pltpu.CompilerParams(
                vmem_limit_bytes=100 * 2**20, disable_bounds_checks=True, flags=flags),
        )(ax.reshape(B, D), r(ak), r(av), w(awq), w(awo.T), bx.reshape(B, D), r(bk), r(bv), w(bwq), w(bwo.T))
        return out.reshape(B, 1, 2 * D)
    return jax.jit(f)


_kernel = build(tshape=(48, 1))


@jax.jit
def pallas_concat_heads__gqa_block_cached__gqa_block_cached__decode_kernel(
        A_x, A_k_cache, A_v_cache, A_wq, A_wo, B_x, B_k_cache, B_v_cache, B_wq, B_wo):
    return _kernel(A_x, A_k_cache, A_v_cache, A_wq, A_wo, B_x, B_k_cache, B_v_cache, B_wq, B_wo)
```

```python
import jax
import jax.numpy as jnp
import jax.experimental.pallas as pl
import jax.experimental.pallas.tpu as pltpu

B, D, HQ, HKV, SK, DH = 2, 576, 32, 16, 4096, 128
F32, BF16 = jnp.float32, jnp.bfloat16
NT = (((1,), (1,)), ((), ()))


def build(SR=256, LA=9, NB=4, perm=(0, 4, 1, 5, 2, 6, 3, 7), yord=(0, 4, 2, 6, 1, 5, 3, 7),
          qm=(0, 2, 1, 3), qx=(0, 1, 2, 3), qy=(0, 1, 2, 3, 4, 5, 6, 7), scoped=True, nosem=False, nobounds=False,
          compute=True, flags=None):
    ROWS = 64
    G = 8
    SH = G * HKV // HQ
    NG = HQ // G
    GW = G * DH
    NR = SK // SR
    NA = B * NR
    P, R = 9, 64
    L = R // 8
    WIN = L + 1
    NCH = 4 * NG
    SCALE = DH ** -0.5

    def body(ax, ak, av, awq, awo, bx, bk, bv, bwq, bwo, finish,
             xbuf, wqbuf, wobuf, midbuf, kvbuf, q_scr, s_scr, m_scr, o_scr, acc_scr, res,
             xsem, wqsem, wosem, kvsem):
        def wait_all(ref, sem):
            pltpu.make_async_copy(ref, ref, sem).wait()

        def start_kv(src, j):
            slot = jax.lax.rem(j, WIN)
            b = jax.lax.rem(jax.lax.div(j, NR), B)
            r0 = pl.multiple_of(jax.lax.rem(j, NR) * SR, SR)
            for r in range(0, SR, ROWS):
                for i, g in enumerate(perm):
                    pltpu.make_async_copy(
                        src.at[b, pl.ds(2 * g, 2), pl.ds(r0 + r, ROWS)],
                        kvbuf.at[slot, pl.ds(2 * g, 2), pl.ds(r, ROWS)],
                        kvsem.at[slot]).start(priority=i % 2)

        def rows8(y):
            return pl.ds(pl.multiple_of(jnp.int32(8) * y, 8), 8)

        @pl.loop(0, L)
        def _(i):
            y = i
            if qy[1] == 4:
                y = (i & 1) * 4 + (i & 2) + (i >> 2)
            for x in qx:
                for m in qm + (None,):
                    for br, w in enumerate((awq, bwq)):
                        if m is not None:
                            idx = (pl.ds(2 * m + br, 2), rows8(y), pl.ds(x * GW, GW))
                        elif x % 2 == 0:
                            idx = ((P - 1) * (1 - br), rows8(y), pl.ds(x * GW, 2 * GW))
                        else:
                            continue
                        pltpu.make_async_copy(w.at[idx], wqbuf.at[br].at[idx], wqsem.at[0]).start(priority=br)

        x_copies = [pltpu.make_async_copy(x, xbuf.at[br], xsem.at[br]) for br, x in enumerate((ax, bx))]
        for br, c in enumerate(x_copies):
            c.start(priority=br)

        @pl.loop(0, L - NG)
        def _(j):
            start_kv(ak, j)

        o_scr[...] = jnp.zeros(o_scr.shape, F32)
        acc_scr[...] = jnp.zeros(acc_scr.shape, F32)
        for c in x_copies:
            c.wait()
        wait_all(wqbuf, wqsem.at[0])

        row = jax.lax.broadcasted_iota(jnp.int32, (B * G, DH), 0)
        rowd = jax.lax.broadcasted_iota(jnp.int32, (B * G, D), 0)
        xs = []
        for br in range(2):
            x = xbuf[br].astype(F32)
            xs.append(jnp.where(rowd < G, x[0:1, :], x[1:2, :]).astype(BF16))

        @pl.loop(0, NG)
        def _(g):
            start_kv(ak, L - NG + g)
            for br in range(2 if compute else 0):
                q = None
                for t in range(G):
                    cols = pl.ds(pl.multiple_of(g * GW + t * DH, DH), DH)
                    r = jnp.dot(xs[br], wqbuf[br, :, :, cols].reshape(D, DH), preferred_element_type=F32)
                    q = r if q is None else jnp.where(row % G == t, r, q)
                for b in range(B):
                    q_scr[br * B + b, g] = q[b * G:(b + 1) * G]

        def scores(j, ms):
            slot = jax.lax.rem(j, WIN)
            wait_all(kvbuf.at[slot], kvsem.at[slot])
            if not compute:
                return ms
            u = jax.lax.div(j, NR)
            first = jax.lax.rem(j, NR) == 0
            head = jax.lax.broadcasted_iota(jnp.int32, (G, SR), 0) // (G // SH)
            new = []
            for g in range(NG):
                q = q_scr[u, g].astype(BF16)
                s = None
                for h in range(SH):
                    r = jax.lax.dot_general(q, kvbuf[slot, g * SH + h], NT, preferred_element_type=F32)
                    s = r if s is None else jnp.where(head == h, r, s)
                s = s * SCALE
                s_scr[j, g] = s
                m = jnp.where(first, -jnp.inf, ms[g])
                for t in range(0, SR, DH):
                    m = jnp.maximum(m, s[:, t:t + DH])
                m_scr[u, g] = m
                new.append(m)
            return tuple(new)

        def values(j, carry):
            slot = jax.lax.rem(j, WIN)
            wait_all(kvbuf.at[slot], kvsem.at[slot])
            if not compute:
                return carry
            jk = j - 2 * NA
            u = jax.lax.div(jk, NR)
            first = jax.lax.rem(jk, NR) == 0
            head = jax.lax.broadcasted_iota(jnp.int32, (G, DH), 0) // (G // SH)
            new = []
            for g in range(NG):
                l, a = carry[g]
                p = jnp.exp(s_scr[jk, g] - jnp.max(m_scr[u, g], axis=1, keepdims=True))
                l = jnp.where(first, 0.0, l)
                for t in range(0, SR, DH):
                    l = l + p[:, t:t + DH]
                p = p.astype(BF16)
                o = None
                for h in range(SH):
                    r = jnp.dot(p, kvbuf[slot, g * SH + h], preferred_element_type=F32)
                    o = r if o is None else jnp.where(head == h, r, o)
                a = jnp.where(first, 0.0, a) + o
                o_scr[pl.ds(g * G * 8 + u, G, stride=8), :] = a / jnp.sum(l, axis=1, keepdims=True)
                new.append((l, a))
            return tuple(new)

        def run(step, lo, hi, src, carry):
            def one(j, c):
                start_kv(src, j + L)
                return step(j, c)
            return jax.lax.fori_loop(lo, hi, one, carry)

        z = jnp.zeros((G, DH), F32)
        ms = run(scores, 0, NA - L, ak, (z,) * NG)
        ms = run(scores, NA - L, 2 * NA - L, bk, ms)
        run(scores, 2 * NA - L, 2 * NA, av, ms)
        carry = run(values, 2 * NA, 3 * NA - L, av, ((z, z),) * NG)
        carry = run(values, 3 * NA - L, 4 * NA - L, bv, carry)

        def start_wo(k, y):
            k = jnp.int32(k)
            m, x = jax.lax.rem(k, 4), jax.lax.div(k, 4)
            for br, w in enumerate((awo, bwo)):
                pltpu.make_async_copy(
                    w.at[pl.ds(2 * m + br, 2), rows8(y), pl.ds(pl.multiple_of(x * GW, GW), GW)],
                    wobuf.at[k, br, :, rows8(y)], wosem.at[k]).start(priority=br)

        def last_values(i, c):
            for x in range(0, HQ * DH, 2 * GW):
                for br, w in enumerate((awo, bwo)):
                    idx = (rows8(i), pl.ds(x, 2 * GW))
                    pltpu.make_async_copy(w.at[(P - 1) * (1 - br)].at[idx], midbuf.at[br].at[idx],
                                          wosem.at[NCH]).start(priority=br)
            for k in range(NB):
                start_wo(k, i)
            return values(4 * NA - L + i, c)
        jax.lax.fori_loop(0, L, last_values, carry)

        @pl.loop(0, L)
        def _(y):
            for k in range(NB, LA - 1):
                start_wo(k, y)

        def heads(x):
            return [o_scr[pl.ds(pl.multiple_of(jnp.int32(x * G + t) * 8, 8), 8)].astype(BF16) for t in range(G)]

        def project(a, os, w_cols):
            for t in range(G if compute else 0):
                a = a + jax.lax.dot_general(os[t], w_cols(t).reshape(DH, DH), NT, preferred_element_type=F32)
            return a

        wait_all(midbuf, wosem.at[NCH])

        @pl.loop(0, NG)
        def _(x):
            for y in range(L // NG):
                start_wo(LA - 1, (L // NG) * x + y)
            acc_scr[4] = project(
                acc_scr[4], heads(x), lambda t: midbuf[:, :, pl.ds(pl.multiple_of(x * GW + t * DH, DH), DH)])

        def chunk(k):
            m, x = jax.lax.rem(k, 4), jax.lax.div(k, 4)
            wait_all(wobuf.at[k], wosem.at[k])
            os = heads(x)
            for br in range(2):
                n = m + 5 * br
                acc_scr[n] = project(acc_scr[n], os, lambda t: wobuf[k, br, :, :, t * DH:(t + 1) * DH])

        @pl.loop(0, NCH - LA)
        def _(k):
            for y in yord:
                start_wo(k + LA, y)
            chunk(k)

        pl.loop(NCH - LA, NCH - 1)(chunk)

        def emit(n, a):
            col = n * DH + jax.lax.broadcasted_iota(jnp.int32, (B, DH), 1)
            res[:, n * DH:(n + 1) * DH] = jnp.where(col < D, a[0:B], a[B:2 * B]).astype(BF16)

        last = (3, 8)
        for n in range(P):
            if n not in last:
                emit(n, acc_scr[n])
        os = heads(NG - 1)
        prev = [acc_scr[n] for n in last]
        wait_all(wobuf.at[NCH - 1], wosem.at[NCH - 1])
        for br, n in enumerate(last):
            emit(n, project(prev[br], os, lambda t: wobuf[NCH - 1, br, :, :, t * DH:(t + 1) * DH]))
        finish()

    sems = [pltpu.SemaphoreType.DMA((n,)) for n in (2, 1, NCH + 1, WIN)]

    def kernel(*refs):
        ins, out, scratch = refs[:10], refs[10], refs[11:]
        if scoped:
            store = pltpu.make_async_copy(scratch[-2], out, scratch[-1].at[0])
            pl.run_scoped(lambda *s: body(*ins, store.start, *scratch[:-1], *s), *sems)
            store.wait()
        else:
            body(*ins, lambda: None, *scratch[:-4], out, *scratch[-4:])

    def call(ax, ak, av, awq, awo, bx, bk, bv, bwq, bwo):
        def slabs(t):
            return t.reshape(P, R, HQ * DH)
        hbm = pl.BlockSpec(memory_space=pltpu.HBM)
        scratch = [
            pltpu.VMEM((2, B, D), BF16),
            pltpu.VMEM((2, P, R, HQ * DH), BF16),
            pltpu.VMEM((NCH, 2, 2, R, GW), BF16),
            pltpu.VMEM((2, R, HQ * DH), BF16),
            pltpu.VMEM((WIN, HKV, SR, DH), BF16),
            pltpu.VMEM((2 * B, NG, G, DH), F32),
            pltpu.VMEM((2 * NA, NG, G, SR), F32),
            pltpu.VMEM((2 * B, NG, G, DH), F32),
            pltpu.VMEM((HQ * 8, DH), F32),
            pltpu.VMEM((P, 8, DH), F32),
        ]
        scratch += [pltpu.VMEM((B, 2 * D), BF16), pltpu.SemaphoreType.DMA((1,))] if scoped else sems
        out = pl.pallas_call(
            kernel,
            out_shape=jax.ShapeDtypeStruct((B, 2 * D), BF16),
            in_specs=[hbm] * 10,
            out_specs=hbm if scoped else pl.BlockSpec(),
            scratch_shapes=scratch,
            compiler_params=pltpu.CompilerParams(
                vmem_limit_bytes=96 * 2**20, disable_bounds_checks=nobounds,
                disable_semaphore_checks=nosem, flags=flags),
        )(ax.reshape(B, D), ak, av, slabs(awq), slabs(awo.T), bx.reshape(B, D), bk, bv, slabs(bwq), slabs(bwo.T))
        return out.reshape(B, 1, 2 * D)
    return jax.jit(call)


_kernel = build(qx=(0, 2, 1, 3))


@jax.jit
def pallas_concat_heads__gqa_block_cached__gqa_block_cached__decode_kernel(
        A_x, A_k_cache, A_v_cache, A_wq, A_wo, B_x, B_k_cache, B_v_cache, B_wq, B_wo):
    return _kernel(A_x, A_k_cache, A_v_cache, A_wq, A_wo, B_x, B_k_cache, B_v_cache, B_wq, B_wo)
```

```python
import jax
import jax.numpy as jnp
import jax.experimental.pallas as pl
import jax.experimental.pallas.tpu as pltpu

B, D, HQ, HKV, SK, DH = 2, 576, 32, 16, 4096, 128
F32, BF16 = jnp.float32, jnp.bfloat16
NT = (((1,), (1,)), ((), ()))
SCALE = DH ** -0.5

G = 8
SH = G * HKV // HQ
NG = HQ // G
GW = G * DH

SR = 256
ROWS = 64
HEAD_PAIRS = (0, 4, 1, 5, 2, 6, 3, 7)
NR = SK // SR
NA = B * NR

P, R = 9, 64
ROW_TILES = (0, 4, 2, 6, 1, 5, 3, 7)
L = R // 8
WIN = L + 1

NCH = 4 * NG
NB = 4
LA = 9
TAIL = ((NCH - 2, 0, 0, G), (NCH - 2, 1, 0, G),
        (NCH - 1, 0, 0, G // 2), (NCH - 1, 0, G // 2, G // 2),
        (NCH - 1, 1, 0, G // 2), (NCH - 1, 1, G // 2, G // 2))


def _divmod(i, n):
    if isinstance(i, int):
        return divmod(i, n)
    return jax.lax.div(i, n), jax.lax.rem(i, n)


def _block(i, n):
    return pl.ds(i * n if isinstance(i, int) else pl.multiple_of(i * n, n), n)


def _wait_all(ref, sem):
    pltpu.make_async_copy(ref, ref, sem).wait()


def _compute(ax, ak, av, awq, awo, bx, bk, bv, bwq, bwo,
             xbuf, wqbuf, wobuf, midbuf, kvbuf, q_scr, s_scr, m_scr, o_scr, acc_scr, res,
             xsem, wqsem, wosem, tailsem, kvsem):
    def start_kv(src, j):
        slot = jax.lax.rem(j, WIN)
        u, step = _divmod(j, NR)
        b = jax.lax.rem(u, B)
        r0 = pl.multiple_of(step * SR, SR)
        for r in range(0, SR, ROWS):
            for i, g in enumerate(HEAD_PAIRS):
                pltpu.make_async_copy(
                    src.at[b, pl.ds(2 * g, 2), pl.ds(r0 + r, ROWS)],
                    kvbuf.at[slot, pl.ds(2 * g, 2), pl.ds(r, ROWS)],
                    kvsem.at[slot]).start(priority=i % 2)

    @pl.loop(0, R // 8)
    def _(y):
        for x in range(NG):
            for m in (0, 2, 1, 3, None):
                for br, w in enumerate((awq, bwq)):
                    if m is not None:
                        idx = (pl.ds(2 * m + br, 2), _block(y, 8), _block(x, GW))
                    elif x % 2 == 0:
                        idx = ((P - 1) * (1 - br), _block(y, 8), _block(x // 2, 2 * GW))
                    else:
                        continue
                    pltpu.make_async_copy(w.at[idx], wqbuf.at[(br,) + idx], wqsem.at[0]).start(priority=br)

    x_copies = [pltpu.make_async_copy(x, xbuf.at[br], xsem.at[br]) for br, x in enumerate((ax, bx))]
    for br, c in enumerate(x_copies):
        c.start(priority=br)

    @pl.loop(0, L - NG)
    def _(j):
        start_kv(ak, j)

    o_scr[...] = jnp.zeros(o_scr.shape, F32)
    acc_scr[...] = jnp.zeros(acc_scr.shape, F32)
    for c in x_copies:
        c.wait()
    _wait_all(wqbuf, wqsem.at[0])

    row = jax.lax.broadcasted_iota(jnp.int32, (B * G, DH), 0)
    rowd = jax.lax.broadcasted_iota(jnp.int32, (B * G, D), 0)
    xs = []
    for br in range(2):
        x = xbuf[br].astype(F32)
        xs.append(jnp.where(rowd < G, x[0:1, :], x[1:2, :]).astype(BF16))

    @pl.loop(0, NG)
    def _(g):
        start_kv(ak, L - NG + g)
        for br in range(2):
            q = None
            for t in range(G):
                w = wqbuf[br, :, :, _block(g * G + t, DH)].reshape(D, DH)
                r = jnp.dot(xs[br], w, preferred_element_type=F32)
                q = r if q is None else jnp.where(row % G == t, r, q)
            for b in range(B):
                q_scr[br * B + b, g] = q[b * G:(b + 1) * G]

    def scores(j, ms):
        slot = jax.lax.rem(j, WIN)
        _wait_all(kvbuf.at[slot], kvsem.at[slot])
        u, step = _divmod(j, NR)
        head = jax.lax.broadcasted_iota(jnp.int32, (G, SR), 0) // (G // SH)
        new = []
        for g in range(NG):
            q = q_scr[u, g].astype(BF16)
            s = None
            for h in range(SH):
                r = jax.lax.dot_general(q, kvbuf[slot, g * SH + h], NT, preferred_element_type=F32)
                s = r if s is None else jnp.where(head == h, r, s)
            s = s * SCALE
            s_scr[j, g] = s
            m = jnp.where(step == 0, -jnp.inf, ms[g])
            for t in range(0, SR, DH):
                m = jnp.maximum(m, s[:, t:t + DH])
            m_scr[u, g] = m
            new.append(m)
        return tuple(new)

    def values(j, carry):
        slot = jax.lax.rem(j, WIN)
        _wait_all(kvbuf.at[slot], kvsem.at[slot])
        jk = j - 2 * NA
        u, step = _divmod(jk, NR)
        head = jax.lax.broadcasted_iota(jnp.int32, (G, DH), 0) // (G // SH)
        new = []
        for g in range(NG):
            l, a = carry[g]
            p = jnp.exp(s_scr[jk, g] - jnp.max(m_scr[u, g], axis=1, keepdims=True))
            l = jnp.where(step == 0, 0.0, l)
            for t in range(0, SR, DH):
                l = l + p[:, t:t + DH]
            p = p.astype(BF16)
            o = None
            for h in range(SH):
                r = jnp.dot(p, kvbuf[slot, g * SH + h], preferred_element_type=F32)
                o = r if o is None else jnp.where(head == h, r, o)
            a = jnp.where(step == 0, 0.0, a) + o
            o_scr[pl.ds(g * G * 8 + u, G, stride=8), :] = a / jnp.sum(l, axis=1, keepdims=True)
            new.append((l, a))
        return tuple(new)

    def run(step_fn, lo, hi, src, carry):
        def one(j, c):
            start_kv(src, j + L)
            return step_fn(j, c)
        return jax.lax.fori_loop(lo, hi, one, carry)

    z = jnp.zeros((G, DH), F32)
    ms = run(scores, 0, NA - L, ak, (z,) * NG)
    ms = run(scores, NA - L, 2 * NA - L, bk, ms)
    run(scores, 2 * NA - L, 2 * NA, av, ms)
    carry = run(values, 2 * NA, 3 * NA - L, av, ((z, z),) * NG)
    carry = run(values, 3 * NA - L, 4 * NA - L, bv, carry)

    wo = (awo, bwo)

    def start_wo(k, y):
        x, m = _divmod(k, 4)
        for br in range(2):
            pltpu.make_async_copy(
                wo[br].at[pl.ds(2 * m + br, 2), _block(y, 8), _block(x, GW)],
                wobuf.at[k, br, :, _block(y, 8)], wosem.at[k]).start(priority=br)

    def last_values(y, c):
        for x in range(NG // 2):
            for br in range(2):
                idx = (_block(y, 8), _block(x, 2 * GW))
                pltpu.make_async_copy(wo[br].at[((P - 1) * (1 - br),) + idx], midbuf.at[(br,) + idx],
                                      wosem.at[NCH]).start(priority=br)
        for k in range(NB):
            start_wo(k, y)
        return values(4 * NA - L + y, c)
    jax.lax.fori_loop(0, L, last_values, carry)

    @pl.loop(0, R // 8)
    def _(y):
        for k in range(NB, LA - 1):
            start_wo(k, y)

    def heads(x):
        return [o_scr[_block(x * G + t, 8)].astype(BF16) for t in range(G)]

    def project(o, w):
        return jax.lax.dot_general(o, w.reshape(DH, DH), NT, preferred_element_type=F32)

    _wait_all(midbuf, wosem.at[NCH])

    @pl.loop(0, NG)
    def _(x):
        for y in range(R // 8 // NG):
            start_wo(LA - 1, (R // 8 // NG) * x + y)
        a = acc_scr[4]
        for t, o in enumerate(heads(x)):
            a = a + project(o, midbuf[:, :, _block(x * G + t, DH)])
        acc_scr[4] = a

    def chunk(k):
        x, m = _divmod(k, 4)
        _wait_all(wobuf.at[k], wosem.at[k])
        os = heads(x)
        for br in range(2):
            a = acc_scr[m + 5 * br]
            for t in range(G):
                a = a + project(os[t], wobuf[k, br, :, :, _block(t, DH)])
            acc_scr[m + 5 * br] = a

    first_tail = TAIL[0][0]

    @pl.loop(0, first_tail - LA)
    def _(k):
        for y in ROW_TILES:
            start_wo(k + LA, y)
        chunk(k)

    for i, (k, br, t0, nt) in enumerate(TAIL):
        x, m = divmod(k, 4)
        for n, y in enumerate(ROW_TILES):
            pltpu.make_async_copy(
                wo[br].at[pl.ds(2 * m + br, 2), _block(y, 8), pl.ds(x * GW + t0 * DH, nt * DH)],
                wobuf.at[k, br, :, _block(y, 8), pl.ds(t0 * DH, nt * DH)],
                tailsem.at[i]).start(priority=n % 2)

    pl.loop(first_tail - LA, first_tail)(chunk)

    def emit(n, a):
        col = n * DH + jax.lax.broadcasted_iota(jnp.int32, (B, DH), 1)
        res[:, _block(n, DH)] = jnp.where(col < D, a[0:B], a[B:2 * B]).astype(BF16)

    open_tiles = [k % 4 + 5 * br for k, br, _, _ in TAIL]
    acc = []
    for n in range(P):
        acc.append(acc_scr[n])
        if n not in open_tiles:
            emit(n, acc[n])
    os = heads(NG - 1)
    for i, (k, br, t0, nt) in enumerate(TAIL):
        n = open_tiles[i]
        _wait_all(wobuf.at[k, br, :, :, pl.ds(t0 * DH, nt * DH)], tailsem.at[i])
        for t in range(t0, t0 + nt):
            acc[n] = acc[n] + project(os[t], wobuf[k, br, :, :, _block(t, DH)])
        if t0 + nt == G:
            emit(n, acc[n])


def _kernel(*refs):
    ins, out, scratch, outsem = refs[:10], refs[10], refs[11:-1], refs[-1]
    store = pltpu.make_async_copy(scratch[-1], out, outsem.at[0])

    def scoped(*sems):
        _compute(*ins, *scratch, *sems)
        store.start()

    pl.run_scoped(scoped, *[pltpu.SemaphoreType.DMA((n,)) for n in (2, 1, NCH + 1, len(TAIL), WIN)])
    store.wait()


@jax.jit
def pallas_concat_heads__gqa_block_cached__gqa_block_cached__decode_kernel(
    A_x: jax.Array,
    A_k_cache: jax.Array,
    A_v_cache: jax.Array,
    A_wq: jax.Array,
    A_wo: jax.Array,
    B_x: jax.Array,
    B_k_cache: jax.Array,
    B_v_cache: jax.Array,
    B_wq: jax.Array,
    B_wo: jax.Array,
):
    def slabs(w):
        return w.reshape(P, R, HQ * DH)

    hbm = pl.BlockSpec(memory_space=pltpu.HBM)
    out = pl.pallas_call(
        _kernel,
        out_shape=jax.ShapeDtypeStruct((B, 2 * D), BF16),
        in_specs=[hbm] * 10,
        out_specs=hbm,
        scratch_shapes=[
            pltpu.VMEM((2, B, D), BF16),
            pltpu.VMEM((2, P, R, HQ * DH), BF16),
            pltpu.VMEM((NCH, 2, 2, R, GW), BF16),
            pltpu.VMEM((2, R, HQ * DH), BF16),
            pltpu.VMEM((WIN, HKV, SR, DH), BF16),
            pltpu.VMEM((2 * B, NG, G, DH), F32),
            pltpu.VMEM((2 * NA, NG, G, SR), F32),
            pltpu.VMEM((2 * B, NG, G, DH), F32),
            pltpu.VMEM(((HQ + 1) * 8, DH), F32),
            pltpu.VMEM((P, 8, DH), F32),
            pltpu.VMEM((B, 2 * D), BF16),
            pltpu.SemaphoreType.DMA((1,)),
        ],
        compiler_params=pltpu.CompilerParams(
            vmem_limit_bytes=64 * 2**20,
            flags={"XLA_TPU_RESCHEDULE_DMA_DONES": True},
        ),
    )(A_x.reshape(B, D), A_k_cache, A_v_cache, slabs(A_wq), slabs(A_wo.T),
      B_x.reshape(B, D), B_k_cache, B_v_cache, slabs(B_wq), slabs(B_wo.T))
    return out.reshape(B, 1, 2 * D)
```
